```python
import os as _os
_os.environ.setdefault("JAX_PLATFORMS", "cpu")
import jax
import jax.numpy as jnp

def _softmax(x, axis=-1):
    return jax.nn.softmax(x, axis=axis)
def _gelu(x):
    return jax.nn.gelu(x, approximate=True)
def _silu(x):
    return jax.nn.silu(x)
def _sigmoid(x):
    return jax.nn.sigmoid(x)
def _layernorm(x, axis=-1, eps=1e-5):
    m = jnp.mean(x, axis=axis, keepdims=True)
    v = jnp.var(x, axis=axis, keepdims=True)
    return (x - m) / jnp.sqrt(v + eps)
def _scatter_add(tgt, idx, src, axis=0):
    return tgt.at[idx].add(src)
def _segment_sum(src, seg, n):
    return jax.ops.segment_sum(src, seg, n)
class _Rng:
    def __init__(self, key):
        self._k = key
    def _next(self):
        self._k, sub = jax.random.split(self._k)
        return sub
    def normal(self, shape):
        return jax.random.normal(self._next(), shape, dtype=jnp.bfloat16)
    def randint(self, lo, hi, shape):
        return jax.random.randint(self._next(), shape, lo, hi, dtype=jnp.int32)
    def uniform(self, shape, lo=0.0, hi=1.0):
        return jax.random.uniform(self._next(), shape, jnp.bfloat16, lo, hi)
    def permutation(self, n):
        return jax.random.permutation(self._next(), n)


kernel_name = 'concat_heads__mha_block_cached__mha_block_cached__near_ridge'

def setup_inputs():
    _rng = _Rng(jax.random.key(int.from_bytes(__import__("os").urandom(4), "little")))
    _w = (lambda a: (lambda t: t.astype(jnp.bfloat16) if jnp.issubdtype(t.dtype, jnp.floating) else t)(jnp.asarray(a)))
    def _A_setup():
        B, Sq, D = 16, 192, 512
        H, Sk, Dh = 32, 512, 128
        return {
            "x": _w((lambda *s: _rng.normal(s) * 0.8)(B, Sq, D)),
            "k_cache": _w((lambda *s: _rng.normal(s) * 0.8)(B, H, Sk, Dh)),
            "v_cache": _w((lambda *s: _rng.normal(s) * 0.05)(B, H, Sk, Dh)),
            "wq": _w((lambda *s: _rng.normal(s) * 0.8)(D, H * Dh) * (D ** -0.5)),
            "wo": _w((lambda *s: _rng.normal(s) * 0.05)(H * Dh, D) * ((H * Dh) ** -0.5)),
        }
    _A_in = _A_setup()

    def _B_setup():
        B, Sq, D = 16, 192, 512
        H, Sk, Dh = 32, 512, 128
        return {
            "x": _w((lambda *s: _rng.normal(s) * 0.8)(B, Sq, D)),
            "k_cache": _w((lambda *s: _rng.normal(s) * 0.8)(B, H, Sk, Dh)),
            "v_cache": _w((lambda *s: _rng.normal(s) * 0.05)(B, H, Sk, Dh)),
            "wq": _w((lambda *s: _rng.normal(s) * 0.8)(D, H * Dh) * (D ** -0.5)),
            "wo": _w((lambda *s: _rng.normal(s) * 0.05)(H * Dh, D) * ((H * Dh) ** -0.5)),
        }
    _B_in = _B_setup()

    return {
        "A_x": _A_in["x"],
        "A_k_cache": _A_in["k_cache"],
        "A_v_cache": _A_in["v_cache"],
        "A_wq": _A_in["wq"],
        "A_wo": _A_in["wo"],
        "B_x": _B_in["x"],
        "B_k_cache": _B_in["k_cache"],
        "B_v_cache": _B_in["v_cache"],
        "B_wq": _B_in["wq"],
        "B_wo": _B_in["wo"],
    }

def reference(A_x, A_k_cache, A_v_cache, A_wq, A_wo, B_x, B_k_cache, B_v_cache, B_wq, B_wo):
    def _A_ref(x, k_cache, v_cache, wq, wo):
        B, Sq, D = x.shape
        H, Dh = 32, 128
        q = (lambda x, *d: x.transpose(*d))((x @ wq).reshape(B, Sq, H, Dh), 0, 2, 1, 3)
        scores = jnp.einsum("bhqd,bhkd->bhqk", q, k_cache) * (Dh ** -0.5)
        p = _softmax(scores, axis=-1)
        o = jnp.einsum("bhqk,bhkd->bhqd", p, v_cache)
        return (lambda x, *d: x.transpose(*d))(o, 0, 2, 1, 3).reshape(B, Sq, H * Dh) @ wo

    def _B_ref(x, k_cache, v_cache, wq, wo):
        B, Sq, D = x.shape
        H, Dh = 32, 128
        q = (lambda x, *d: x.transpose(*d))((x @ wq).reshape(B, Sq, H, Dh), 0, 2, 1, 3)
        scores = jnp.einsum("bhqd,bhkd->bhqk", q, k_cache) * (Dh ** -0.5)
        p = _softmax(scores, axis=-1)
        o = jnp.einsum("bhqk,bhkd->bhqd", p, v_cache)
        return (lambda x, *d: x.transpose(*d))(o, 0, 2, 1, 3).reshape(B, Sq, H * Dh) @ wo

    a = _A_ref(A_x, A_k_cache, A_v_cache, A_wq, A_wo)
    b = _B_ref(B_x, B_k_cache, B_v_cache, B_wq, B_wo)
    return jnp.concatenate([a, b], axis=-1)
```

```python
import functools

import jax
import jax.numpy as jnp
from jax import lax
import jax.experimental.pallas as pl
import jax.experimental.pallas.tpu as pltpu

LOG2E = 1.4426950408889634
NT = (((1,), (1,)), ((), ()))
f32 = jnp.float32
bf16 = jnp.bfloat16

P = 2
HB = 16
NS = 4
PD = 2
DQ = 5
Q0_PARTS = (1, 4, 9, 16)
WB_AT = 7
STEP_ORDER = ("s0", "p0", "s1", "q", "p1", "o")
STEP_ORDER_Q_READY = ("p1", "o", "s1", "p0", "s0")


def _log2(n):
    assert n & (n - 1) == 0
    return n.bit_length() - 1


def _kernel(ax, ak, av, awq, awo, bx, bk, bv, bwq, bwo, out,
            wq_s, wo_s, xq_s, x_s, kv_s, q_s, acc_s, oc_s, ob_s, sems,
            *, B, Sq, D, H, Sk, Dh):
    NH = H // HB
    NG = B // P
    NB = 2 * NG * NH
    NGG = 2 * NG
    M = P * Sq
    lNH, lNG = _log2(NH), _log2(NG)
    c_scale = (Dh ** -0.5) * LOG2E
    X = (ax, bx)
    KV = ((ak, av), (bk, bv))
    WQ = (awq, bwq)
    WO = (awo, bwo)
    GQ = (DQ - 1) >> lNH
    NP0 = len(Q0_PARTS)
    assert NH == 2 and PD == NH and NH <= DQ <= WB_AT < NG * NH and GQ >= 1 and Q0_PARTS[-1] == HB

    o_wb = 0
    o_o = 1
    o_kv = 2
    o_xq = o_kv + NS
    o_wq = o_xq + GQ + 1
    o_wo = o_wq + NP0 + 1

    def dec(tb):
        hh = tb & (NH - 1)
        gg = tb >> lNH
        return hh, gg, gg >> lNG, gg & (NG - 1)

    def x_cp(dst, ab, g, sem):
        return pltpu.make_async_copy(X[ab].at[pl.ds(g * P, P)], dst, sem)

    def kv_cp(which, ab, g, hh, slot):
        return pltpu.make_async_copy(KV[ab][which].at[pl.ds(g * P, P), pl.ds(hh * HB, HB)],
                                     kv_s.at[slot, which], sems.at[o_kv + slot])

    def wq_cps(ab, h0, h1, sem):
        return [functools.partial(pltpu.make_async_copy, WQ[ab].at[:, pl.ds(h * Dh, Dh)], wq_s.at[ab, h], sem)
                for h in range(h0, h1)]

    def wo_cp(ab, h0, h1, sem):
        rows = pl.ds(h0 * Dh, (h1 - h0) * Dh)
        return pltpu.make_async_copy(WO[ab].at[rows], wo_s.at[ab, rows], sem)

    def out_cp(ab, g, gg):
        return pltpu.make_async_copy(ob_s.at[gg], out.at[pl.ds(g * P, P), :, pl.ds(ab * D, D)], sems.at[o_o])

    def wait_like(ref, sem):
        pltpu.make_async_copy(ref, ref, sem).wait()

    def xq_cp(gq):
        return x_cp(xq_s.at[gq], 0, gq, sems.at[o_xq + gq])

    def wq_part(k):
        if k < NP0:
            return (0 if k == 0 else Q0_PARTS[k - 1]), Q0_PARTS[k]
        return HB, 2 * HB

    def wq_part_cps(k):
        return wq_cps(0, *wq_part(k), sems.at[o_wq + k])

    def wo_part_cp(b):
        return wo_cp(0, b * HB, (b + 1) * HB, sems.at[o_wo + b])

    def wb_cps():
        return wq_cps(1, 0, H, sems.at[o_wb]) + [functools.partial(wo_cp, 1, 0, H, sems.at[o_wb])]

    def wo_head(ab, head):
        return wo_s[ab, pl.ds(pl.multiple_of(head * Dh, Dh), Dh), :]

    def qproj(x, ab, head):
        q = jnp.dot(x, wq_s[ab, head], preferred_element_type=f32)
        return [(q[p * Sq:(p + 1) * Sq] * c_scale).astype(bf16) for p in range(P)]

    def q_heads(tb, h0, h1):
        hh, gg, _, _ = dec(tb)
        for h in range(h0, h1):
            qs = qproj(xq_s[gg].reshape(M, D), 0, hh * HB + h)
            for p in range(P):
                q_s[tb, h, p] = qs[p]

    xq_cp(0).start()
    for k in range(NP0):
        for cp in wq_part_cps(k):
            cp().start()
    xq_cp(1).start()
    for cp in wq_part_cps(NP0):
        cp().start()
    for gq in range(2, GQ + 1):
        xq_cp(gq).start()
    for tb in range(PD):
        hh, gg, ab, g = dec(tb)
        wo_part_cp(tb).start()
        kv_cp(0, ab, g, hh, tb).start()
        kv_cp(1, ab, g, hh, tb).start()
    acc_s[...] = jnp.zeros_like(acc_s)
    oc_s[...] = jnp.zeros_like(oc_s)

    xq_cp(0).wait()
    for k in range(NP0):
        for cp in wq_part_cps(k):
            cp().wait()
        q_heads(0, *wq_part(k))

    def q_body(i, c):
        tb = jnp.where(i == 1, 2, jnp.where(i == 2, 1, i))
        hh, gg, _, _ = dec(tb)

        @pl.when(tb == 1)
        def _():
            for cp in wq_part_cps(NP0):
                cp().wait()

        @pl.when(hh == 0)
        def _():
            wait_like(xq_s.at[gg], sems.at[o_xq + gg])

        q_heads(tb, 0, HB)
        return c

    lax.fori_loop(1, DQ, q_body, 0)

    def top_scalars(t):
        hh, gg, ab, g = dec(t)
        phh, pgg, pab, _ = dec(jnp.maximum(t - 1, 0))
        phead = phh * HB + HB - 1
        finish = jnp.logical_and(hh == 0, t > 0)
        oslot = jnp.where(finish, pgg, NGG)
        special = jnp.logical_or(t == WB_AT, t == NG * NH).astype(jnp.int32)
        return (hh, ab, t & (NS - 1), pab, phead, oslot, special)

    def block(t, q_ready, sc):
        hh, ab, slot, pab, phead, oslot, special = sc
        tn = t + PD
        nhh, ngg, nab, ng = dec(tn)
        nslot = tn & (NS - 1)
        phh, pgg, _, _ = dec(jnp.maximum(t - 1, 0))

        if q_ready:
            for b in range(NH):
                @pl.when(t == b)
                def _():
                    wo_part_cp(b).wait()
        else:
            @pl.when(special != 0)
            def _():
                @pl.when(t == WB_AT)
                def _():
                    for cp in wb_cps():
                        cp().start()

                @pl.when(t == NG * NH)
                def _():
                    for cp in wb_cps():
                        cp().wait()
        wait_like(kv_s.at[slot, 0], sems.at[o_kv + slot])
        wait_like(kv_s.at[slot, 1], sems.at[o_kv + slot])
        if not q_ready:
            wait_like(x_s.at[slot], sems.at[o_kv + slot])

        out_now = jnp.logical_and(phh == 0, t >= 2)
        cg = pgg - 1

        def start(kind):
            for bb in range(2):
                if kind == "out":
                    cond = jnp.logical_and(out_now, (cg >> lNG) == bb)
                elif kind == "x" and q_ready:
                    cond = jnp.logical_and(nab == bb, tn >= DQ)
                else:
                    cond = nab == bb

                @pl.when(cond)
                def _():
                    if kind == "out":
                        out_cp(bb, cg & (NG - 1), cg).start()
                    elif kind == "x":
                        x_cp(x_s.at[nslot], bb, ng, sems.at[o_kv + nslot]).start()
                    else:
                        kv_cp(kind, bb, ng, nhh, nslot).start()

        pending = ["x", 0, 1, "out"]
        Q, S, O = {}, {}, {}
        acc = [None]

        def do_carry():
            r = jnp.dot(oc_s[...], wo_head(pab, phead), preferred_element_type=f32)
            fin = acc_s[...] + r
            ob_s[oslot] = fin.astype(bf16).reshape(P, Sq, D)
            acc[0] = jnp.where(hh == 0, 0.0, fin)

        def do_q(h):
            if not q_ready:
                qs = qproj(x_s[slot].reshape(M, D), ab, hh * HB + h)
                for p in range(P):
                    Q[h, p] = qs[p]

        def do_s(h, p):
            q = q_s[t, h, p] if q_ready else Q.pop((h, p))
            s = lax.dot_general(q, kv_s[slot, 0, p, h], NT, preferred_element_type=f32)
            S[h, p] = (s, jnp.max(s, axis=-1, keepdims=True))

        def do_pv(h, p):
            if pending:
                start(pending.pop(0))
            s, m = S.pop((h, p))
            e = jnp.exp2(s - m)
            l = jnp.sum(e, axis=-1, keepdims=True)
            o = jnp.dot(e.astype(bf16), kv_s[slot, 1, p, h], preferred_element_type=f32)
            r = pl.reciprocal(l, approx=True)
            r = r * (2.0 - l * r)
            O[h, p] = o * r

        def cat_o(h):
            return jnp.concatenate([O.pop((h, p)) for p in range(P)], axis=0).astype(bf16)

        def do_o(h):
            acc[0] = acc[0] + jnp.dot(cat_o(h), wo_head(ab, hh * HB + h), preferred_element_type=f32)

        if q_ready:
            for p in range(P):
                do_s(0, p)
            do_carry()
        else:
            do_q(0)
            do_carry()
            do_q(1)
            for p in range(P):
                do_s(0, p)
        for h in range(HB):
            for op in (STEP_ORDER_Q_READY if q_ready else STEP_ORDER):
                if op[0] == "s" and h + 1 < HB:
                    do_s(h + 1, int(op[1]))
                if op == "o" and h >= 1:
                    do_o(h - 1)
                if op == "q" and h + 2 < HB:
                    do_q(h + 2)
                if op[0] == "p":
                    do_pv(h, int(op[1]))
        assert not pending
        acc_s[...] = acc[0]
        oc_s[...] = cat_o(HB - 1)

    def ready_body(t, sc):
        block(t, True, sc)
        return top_scalars(t + 1)

    def regular_body(t, sc):
        block(t, False, sc)
        return top_scalars(t + 1)

    sc = lax.fori_loop(0, DQ, ready_body, top_scalars(jnp.int32(0)))
    lax.fori_loop(DQ, NB, regular_body, sc)

    hh, gg, ab, g = dec(NB - 1)
    w = wo_head(ab, hh * HB + HB - 1)
    for p in range(P):
        r = jnp.dot(oc_s[pl.ds(p * Sq, Sq), :], w, preferred_element_type=f32)
        ob_s[gg, p] = (acc_s[pl.ds(p * Sq, Sq), :] + r).astype(bf16)
        pltpu.make_async_copy(ob_s.at[gg, p], out.at[g * P + p, :, pl.ds(ab * D, D)], sems.at[o_o]).start()
    wait_like(ob_s.at[pl.ds(0, NGG)], sems.at[o_o])


@jax.jit
def pallas_concat_heads__mha_block_cached__mha_block_cached__near_ridge_kernel(
    A_x: jax.Array,
    A_k_cache: jax.Array,
    A_v_cache: jax.Array,
    A_wq: jax.Array,
    A_wo: jax.Array,
    B_x: jax.Array,
    B_k_cache: jax.Array,
    B_v_cache: jax.Array,
    B_wq: jax.Array,
    B_wo: jax.Array,
):
    B, Sq, D = A_x.shape
    _, H, Sk, Dh = A_k_cache.shape
    NH = H // HB
    NGG = 2 * B // P
    GQ = (DQ - 1) // NH
    hbm = pl.BlockSpec(memory_space=pl.ANY)
    nsem = 2 + NS + GQ + 1 + len(Q0_PARTS) + 1 + NH
    return pl.pallas_call(
        functools.partial(_kernel, B=B, Sq=Sq, D=D, H=H, Sk=Sk, Dh=Dh),
        in_specs=[hbm] * 10,
        out_specs=hbm,
        out_shape=jax.ShapeDtypeStruct((B, Sq, 2 * D), bf16),
        scratch_shapes=[
            pltpu.VMEM((2, H, D, Dh), bf16),
            pltpu.VMEM((2, H * Dh, D), bf16),
            pltpu.VMEM((GQ + 1, P, Sq, D), bf16),
            pltpu.VMEM((NS, P, Sq, D), bf16),
            pltpu.VMEM((NS, 2, P, HB, Sk, Dh), bf16),
            pltpu.VMEM((DQ, HB, P, Sq, Dh), bf16),
            pltpu.VMEM((P * Sq, D), f32),
            pltpu.VMEM((P * Sq, Dh), bf16),
            pltpu.VMEM((NGG + 1, P, Sq, D), bf16),
            pltpu.SemaphoreType.DMA((nsem,)),
        ],
        compiler_params=pltpu.CompilerParams(
            vmem_limit_bytes=110 * 1024 * 1024,
            disable_bounds_checks=True,
        ),
    )(A_x, A_k_cache, A_v_cache, A_wq, A_wo, B_x, B_k_cache, B_v_cache, B_wq, B_wo)
```
